```python
import jax
import jax.numpy as jnp

def _softmax(x, axis=-1):
    return jax.nn.softmax(x, axis=axis)

def _gelu(x):
    return jax.nn.gelu(x, approximate=True)

def _silu(x):
    return jax.nn.silu(x)

def _sigmoid(x):
    return jax.nn.sigmoid(x)

def _layernorm(x, axis=-1, eps=1e-05):
    m = jnp.mean(x, axis=axis, keepdims=True)
    v = jnp.var(x, axis=axis, keepdims=True)
    return (x - m) / jnp.sqrt(v + eps)

def _scatter_add(tgt, idx, src, axis=0):
    return tgt.at[idx].add(src)

def _segment_sum(src, seg, n):
    return jax.ops.segment_sum(src, seg, n)

class _Rng:

    def __init__(self, key):
        self._k = key

    def _next(self):
        self._k, sub = jax.random.split(self._k)
        return sub

    def normal(self, shape):
        return jax.random.normal(self._next(), shape, dtype=jnp.bfloat16)

    def randint(self, lo, hi, shape):
        return jax.random.randint(self._next(), shape, lo, hi, dtype=jnp.int32)

    def uniform(self, shape, lo=0.0, hi=1.0):
        return jax.random.uniform(self._next(), shape, jnp.bfloat16, lo, hi)

    def permutation(self, n):
        return jax.random.permutation(self._next(), n)
kernel_name = 'concat_heads__compressed_kv_cla__memory_aug_recurrent_mem_tr__prompt'

def setup_inputs():
    _rng = _Rng(jax.random.key(int.from_bytes(__import__("os").urandom(4), "little")))
    _w = lambda a: (lambda t: t.astype(jnp.bfloat16) if jnp.issubdtype(t.dtype, jnp.floating) else t)(jnp.asarray(a))

    def _A_setup():
        B, H, Sq, Sk, D, M = (1, 32, 2048, 2048, 128, 576)
        Dc = 4 * D
        return {'x': _w((lambda *s: _rng.normal(s) * 0.05)(B, Sq, M)), 'c_kv': _w((lambda *s: _rng.normal(s) * 0.05)(B, Sk, Dc)), 'w_q': _w((lambda *s: _rng.normal(s) * 0.05)(M, H, D) * M ** (-0.5)), 'w_uk': _w((lambda *s: _rng.normal(s) * 0.05)(Dc, H, D) * Dc ** (-0.5)), 'w_uv': _w((lambda *s: _rng.normal(s) * 0.05)(Dc, H, D) * Dc ** (-0.5)), 'w_o': _w((lambda *s: _rng.normal(s) * 0.05)(H, D, M) * (H * D) ** (-0.5))}
    _A_in = _A_setup()

    def _B_setup():
        B, S, Dm = (1, 2048, 576)
        H, Dh = (32, 128)
        M, seg = (8, 32)
        seg = min(seg, S)
        S = S // seg * seg
        return {'x': _w((lambda *s: _rng.normal(s) * 0.05)(B, S, Dm)), 'mem0': _w((lambda *s: _rng.normal(s) * 0.05)(B, M, Dm)), 'Wq': _w((lambda *s: _rng.normal(s) * 0.05)(Dm, H, Dh) * Dm ** (-0.5)), 'Wk': _w((lambda *s: _rng.normal(s) * 0.05)(Dm, H, Dh) * Dm ** (-0.5)), 'Wv': _w((lambda *s: _rng.normal(s) * 0.05)(Dm, H, Dh) * Dm ** (-0.5)), 'Wo': _w((lambda *s: _rng.normal(s) * 0.05)(H, Dh, Dm) * (H * Dh) ** (-0.5)), 'seg_len': seg}
    _B_in = _B_setup()
    return {'A_x': _A_in['x'], 'A_c_kv': _A_in['c_kv'], 'A_w_q': _A_in['w_q'], 'A_w_uk': _A_in['w_uk'], 'A_w_uv': _A_in['w_uv'], 'A_w_o': _A_in['w_o'], 'B_x': _B_in['x'], 'B_mem0': _B_in['mem0'], 'B_Wq': _B_in['Wq'], 'B_Wk': _B_in['Wk'], 'B_Wv': _B_in['Wv'], 'B_Wo': _B_in['Wo'], 'B_seg_len': _B_in['seg_len']}

def reference(A_x, A_c_kv, A_w_q, A_w_uk, A_w_uv, A_w_o, B_x, B_mem0, B_Wq, B_Wk, B_Wv, B_Wo, B_seg_len):

    def _A_ref(x, c_kv, w_q, w_uk, w_uv, w_o):
        B, Sq, M = (x.shape[0], x.shape[1], x.shape[2])
        Sk = c_kv.shape[1]
        H, D = (w_q.shape[1], w_q.shape[2])
        q = jnp.einsum('bqm,mhd->bhqd', x, w_q)
        k = jnp.einsum('bkc,chd->bhkd', c_kv, w_uk)
        v = jnp.einsum('bkc,chd->bhkd', c_kv, w_uv)
        scores = jnp.einsum('bhqd,bhkd->bhqk', q, k) * D ** (-0.5)
        off = Sk - Sq
        qi = jnp.arange(Sq)[:, None]
        kj = jnp.arange(Sk)[None, :]
        cmask = kj <= qi + off
        scores = jnp.where(cmask[None, None], scores, -1000000000.0)
        p = _softmax(scores, axis=-1)
        ctx = jnp.einsum('bhqk,bhkd->bhqd', p, v)
        return jnp.einsum('bhqd,hdm->bqm', ctx, w_o)

    def _B_ref(x, mem0, Wq, Wk, Wv, Wo, seg_len):
        B, S, Dm = x.shape
        H, Dh = (Wq.shape[1], Wq.shape[2])
        M = mem0.shape[1]
        scale = Dh ** (-0.5)
        n_seg = S // seg_len
        L = M + seg_len
        idx = jnp.arange(L)
        mask = (idx[:, None] < M) | (idx[:, None] >= idx[None, :])
        mem = mem0
        outs = []
        for s in range(n_seg):
            xs = x[:, s * seg_len:(s + 1) * seg_len, :].copy()
            h = jnp.concatenate([mem, xs], axis=1)
            q = jnp.einsum('btd,dhe->bhte', h, Wq)
            k = jnp.einsum('btd,dhe->bhte', h, Wk)
            v = jnp.einsum('btd,dhe->bhte', h, Wv)
            scores = jnp.einsum('bhqe,bhke->bhqk', q, k) * scale
            scores = jnp.where(mask[None, None], scores, -1000000000.0)
            p = _softmax(scores, axis=-1)
            o = jnp.einsum('bhqk,bhke->bhqe', p, v)
            o = jnp.einsum('bhte,hed->btd', o, Wo)
            mem = o[:, :M, :].copy()
            outs.append(o[:, M:, :])
        return jnp.concatenate(outs, axis=1)
    a = _A_ref(A_x, A_c_kv, A_w_q, A_w_uk, A_w_uv, A_w_o)
    b = _B_ref(B_x, B_mem0, B_Wq, B_Wk, B_Wv, B_Wo, B_seg_len)
    return jnp.concatenate([a, b], axis=-1)
```

```python
import functools
import math

import jax
import jax.numpy as jnp
from jax import lax
from jax.experimental import pallas as pl
from jax.experimental.pallas import tpu as pltpu

F32 = jnp.float32
BF16 = jnp.bfloat16
LOG2E = 1.4426950408889634
NEG = -1e30

S = 2048
DM = 576
DC = 512
H = 32
DH = 128
NMEM = 8
BQ = 256
BK = 512


def _split_pair(w_ref, p, rows):
    u = w_ref[pl.ds(p, rows, stride=H // 2), :]
    lo = pltpu.bitcast(u << 16, F32)
    hi = pltpu.bitcast(u & jnp.uint32(0xFFFF0000), F32)
    return lo, hi


def _kernel(xa_h, ckv_h, wq_h, wuk_h, wuv_h, wo_h,
            xb_h, mem0_h, bwq_h, bwk_h, bwv_h, bwo_h,
            o_ref,
            xa_s, ckv_s, wq_s, wkv_s, wo_s, q_s, k_s, v_s, acc_s,
            bw_s, bwo_s, qkv_s, ob_s,
            wq_ref, wuk_ref, wuv_ref, bwq_ref, bwk_ref, bwv_ref, xb_ref, mem0_ref, sems, *, seg):
    U32 = jnp.uint32
    pairs = [(xa_h, xa_s), (ckv_h, ckv_s), (wuk_h.bitcast(U32), wuk_ref), (wuv_h.bitcast(U32), wuv_ref),
             (wq_h.bitcast(U32), wq_ref), (wo_h, wo_s),
             (bwq_h.bitcast(U32), bwq_ref), (bwk_h.bitcast(U32), bwk_ref), (bwv_h.bitcast(U32), bwv_ref),
             (bwo_h, bwo_s), (xb_h, xb_ref), (mem0_h, mem0_ref)]
    cps = [pltpu.make_async_copy(a, b, sems.at[i]) for i, (a, b) in enumerate(pairs)]
    for cp in cps:
        cp.start()
    for cp in cps[:6]:
        cp.wait()
    acc_s[...] = jnp.zeros_like(acc_s)
    qscale = DH ** -0.5 * LOG2E

    def head(h, carry):
        @pl.when(h % 2 == 0)
        def _():
            p = h // 2
            lo, hi = _split_pair(wq_ref, p, DM)
            wq_s[0] = lo.astype(BF16)
            wq_s[1] = hi.astype(BF16)
            lo, hi = _split_pair(wuk_ref, p, DC)
            wkv_s[0, :, 0:DH] = lo.astype(BF16)
            wkv_s[1, :, 0:DH] = hi.astype(BF16)
            lo, hi = _split_pair(wuv_ref, p, DC)
            wkv_s[0, :, DH:2 * DH] = lo.astype(BF16)
            wkv_s[1, :, DH:2 * DH] = hi.astype(BF16)

        e = h % 2
        wq = wq_s[e]
        wkv = wkv_s[e]
        RB = 512
        for r in range(S // RB):
            rows = pl.ds(r * RB, RB)
            q = jnp.dot(xa_s[rows, :], wq, preferred_element_type=F32)
            q_s[rows, :] = (q * qscale).astype(BF16)
            kv = jnp.dot(ckv_s[rows, :], wkv, preferred_element_type=F32)
            k_s[rows, :] = kv[:, 0:DH].astype(BF16)
            v_s[rows, :] = kv[:, DH:2 * DH].astype(BF16)

        wo = wo_s[pl.ds(pl.multiple_of(h * DH, DH), DH), :]
        for i in range(S // BQ):
            rows = pl.ds(i * BQ, BQ)
            q = q_s[rows, :]
            kend = (i + 1) * BQ
            m = l = acc = None
            k0 = 0
            while k0 < kend:
                w = min(BK, kend - k0)
                s = lax.dot_general(q, k_s[pl.ds(k0, w), :], (((1,), (1,)), ((), ())),
                                    preferred_element_type=F32)
                if k0 + w > i * BQ:
                    row = lax.broadcasted_iota(jnp.int32, (BQ, w), 0) + i * BQ
                    col = lax.broadcasted_iota(jnp.int32, (BQ, w), 1) + k0
                    s = jnp.where(col <= row, s, NEG)
                mb = jnp.max(s, axis=1, keepdims=True)
                v = v_s[pl.ds(k0, w), :]
                if m is None:
                    m = mb
                    p = jnp.exp2(s - m)
                    l = jnp.sum(p, axis=1, keepdims=True)
                    acc = jnp.dot(p.astype(BF16), v, preferred_element_type=F32)
                else:
                    mn = jnp.maximum(m, mb)
                    a = jnp.exp2(m - mn)
                    p = jnp.exp2(s - mn)
                    l = a * l + jnp.sum(p, axis=1, keepdims=True)
                    acc = a * acc + jnp.dot(p.astype(BF16), v, preferred_element_type=F32)
                    m = mn
                k0 += w
            ctx = (acc / l).astype(BF16)
            acc_s[rows, :] += jnp.dot(ctx, wo, preferred_element_type=F32)
        return carry

    lax.fori_loop(0, H, head, 0)
    o_ref[:, 0:DM] = acc_s[...].astype(BF16)

    def relayout(p, carry):
        for j, w_ref in enumerate((bwq_ref, bwk_ref, bwv_ref)):
            lo, hi = _split_pair(w_ref, p, DM)
            base = j * H * DH
            bw_s[:, pl.ds(pl.multiple_of(base + p * 2 * DH, 2 * DH), DH)] = lo.astype(BF16)
            bw_s[:, pl.ds(pl.multiple_of(base + p * 2 * DH + DH, DH), DH)] = hi.astype(BF16)
        return carry

    for cp in cps[6:]:
        cp.wait()
    lax.fori_loop(0, H // 2, relayout, 0)

    L = NMEM + seg
    ri = lax.broadcasted_iota(jnp.int32, (L, L), 0)
    ci = lax.broadcasted_iota(jnp.int32, (L, L), 1)
    mask = (ri < NMEM) | (ri >= ci)

    def step(t, mem):
        rows = pl.ds(pl.multiple_of(t * seg, seg), seg)
        hcat = jnp.concatenate([mem, xb_ref[rows, :].astype(F32)], axis=0)
        qkv = lax.dot_general(hcat, bw_s[...], (((1,), (0,)), ((), ())), preferred_element_type=F32)
        qkv_s[...] = qkv
        for hh in range(H):
            q = (qkv_s[:, pl.ds(hh * DH, DH)] * qscale).astype(BF16).astype(F32)
            k = qkv_s[:, pl.ds(H * DH + hh * DH, DH)].astype(BF16).astype(F32)
            v = qkv_s[:, pl.ds(2 * H * DH + hh * DH, DH)].astype(BF16).astype(F32)
            s = lax.dot_general(q, k, (((1,), (1,)), ((), ())), preferred_element_type=F32)
            s = jnp.where(mask, s, NEG)
            m = jnp.max(s, axis=1, keepdims=True)
            p = jnp.exp2(s - m)
            l = jnp.sum(p, axis=1, keepdims=True)
            o = jnp.dot(p.astype(BF16).astype(F32), v, preferred_element_type=F32) / l
            ob_s[:, pl.ds(hh * DH, DH)] = o.astype(BF16).astype(F32)
        out = lax.dot_general(ob_s[...], bwo_s[...], (((1,), (0,)), ((), ())), preferred_element_type=F32)
        out = out.astype(BF16)
        o_ref[rows, DM:2 * DM] = out[NMEM:, :]
        return out[:NMEM, :].astype(F32)

    lax.fori_loop(0, S // seg, step, mem0_ref[...].astype(F32))


@functools.partial(jax.jit, static_argnames=("B_seg_len",))
def pallas_concat_heads__compressed_kv_cla__memory_aug_recurrent_mem_tr__prompt_kernel(
        A_x, A_c_kv, A_w_q, A_w_uk, A_w_uv, A_w_o,
        B_x, B_mem0, B_Wq, B_Wk, B_Wv, B_Wo, B_seg_len):
    seg = int(B_seg_len)
    L = NMEM + seg
    vm = pl.BlockSpec(memory_space=pltpu.VMEM)
    hbm = pl.BlockSpec(memory_space=pl.ANY)
    U32 = jnp.uint32
    out = pl.pallas_call(
        functools.partial(_kernel, seg=seg),
        out_shape=jax.ShapeDtypeStruct((S, 2 * DM), BF16),
        in_specs=[hbm] * 12,
        out_specs=vm,
        scratch_shapes=[
            pltpu.VMEM((S, DM), BF16),
            pltpu.VMEM((S, DC), BF16),
            pltpu.VMEM((2, DM, DH), BF16),
            pltpu.VMEM((2, DC, 2 * DH), BF16),
            pltpu.VMEM((H * DH, DM), BF16),
            pltpu.VMEM((S, DH), BF16),
            pltpu.VMEM((S, DH), BF16),
            pltpu.VMEM((S, DH), BF16),
            pltpu.VMEM((S, DM), F32),
            pltpu.VMEM((DM, 3 * H * DH), BF16),
            pltpu.VMEM((H * DH, DM), BF16),
            pltpu.VMEM((L, 3 * H * DH), F32),
            pltpu.VMEM((L, H * DH), F32),
            pltpu.VMEM((DM * H // 2, DH), U32),
            pltpu.VMEM((DC * H // 2, DH), U32),
            pltpu.VMEM((DC * H // 2, DH), U32),
            pltpu.VMEM((DM * H // 2, DH), U32),
            pltpu.VMEM((DM * H // 2, DH), U32),
            pltpu.VMEM((DM * H // 2, DH), U32),
            pltpu.VMEM((S, DM), BF16),
            pltpu.VMEM((NMEM, DM), BF16),
            pltpu.SemaphoreType.DMA((12,)),
        ],
        compiler_params=pltpu.CompilerParams(vmem_limit_bytes=120 * 2 ** 20),
    )(A_x.reshape(S, DM), A_c_kv.reshape(S, DC),
      A_w_q.reshape(DM * H, DH), A_w_uk.reshape(DC * H, DH), A_w_uv.reshape(DC * H, DH),
      A_w_o.reshape(H * DH, DM),
      B_x.reshape(S, DM), B_mem0.reshape(NMEM, DM),
      B_Wq.reshape(DM * H, DH), B_Wk.reshape(DM * H, DH), B_Wv.reshape(DM * H, DH),
      B_Wo.reshape(H * DH, DM))
    return out.reshape(1, S, 2 * DM)
```

```python
import functools

import jax
import jax.numpy as jnp
from jax import lax
from jax.experimental import pallas as pl
from jax.experimental.pallas import tpu as pltpu

F32 = jnp.float32
BF16 = jnp.bfloat16
U32 = jnp.uint32
LOG2E = 1.4426950408889634
NEG = -1e30

S = 2048
DM = 576
DC = 512
H = 32
DH = 128
NMEM = 8
BQ = 256
BK = 512
NT = (((1,), (1,)), ((), ()))
NN = (((1,), (0,)), ((), ()))
QSCALE = DH ** -0.5 * LOG2E


def _split(u):
    lo = pltpu.bitcast(u << 16, F32)
    hi = pltpu.bitcast(u & jnp.uint32(0xFFFF0000), F32)
    return lo, hi


def _kernel(xaT_h, ckv_h, wq_h, wuk_h, wuv_h, woT_h,
            xbT_h, mem0_h, bwq_h, bwk_h, bwv_h, bwoT_h,
            o_h,
            xT_s, xa_s, xb_s, ckv_s, woT_s, bwoT_s, mem0_s,
            wq_r, wuk_r, wuv_r, bwq_r, bwk_r, bwv_r,
            wq_s, wkv_s, q_s, k_s, v_s, acc_s,
            bw_s, bwo_s, qkv_s, ob_s, out_s,
            sem_a, sem_b, sem_m, sem_o, *, seg):
    NP = H // 2
    misc = [pltpu.make_async_copy(xaT_h, xT_s.at[0], sem_m.at[0]),
            pltpu.make_async_copy(ckv_h, ckv_s, sem_m.at[1]),
            pltpu.make_async_copy(xbT_h, xT_s.at[1], sem_m.at[2]),
            pltpu.make_async_copy(mem0_h, mem0_s, sem_m.at[3])]

    def pair_copies(p, srcs, dsts, oT_h, oT_s, sem):
        cps = [pltpu.make_async_copy(s_.bitcast(U32).at[:, p, :], d_.at[p], sem.at[p])
               for s_, d_ in zip(srcs, dsts)]
        cps.append(pltpu.make_async_copy(oT_h.at[pl.ds(2 * p, 2)], oT_s.at[pl.ds(2 * p, 2)], sem.at[p]))
        return cps

    def pair_wait(p, dsts, oT_s, sem):
        for d_ in dsts:
            pltpu.make_async_copy(d_.at[p], d_.at[p], sem.at[p]).wait()
        sl = oT_s.at[pl.ds(2 * p, 2)]
        pltpu.make_async_copy(sl, sl, sem.at[p]).wait()

    a_src, a_dst = (wq_h, wuk_h, wuv_h), (wq_r, wuk_r, wuv_r)
    b_src, b_dst = (bwq_h, bwk_h, bwv_h), (bwq_r, bwk_r, bwv_r)
    misc[0].start()
    misc[1].start()
    for cp in pair_copies(0, a_src, a_dst, woT_h, woT_s, sem_a):
        cp.start()
    acc_s[...] = jnp.zeros_like(acc_s)
    misc[0].wait()
    for r in range(S // 256):
        xa_s[pl.ds(r * 256, 256), :] = xT_s[0, :, pl.ds(r * 256, 256)].T
    misc[1].wait()
    pair_wait(0, a_dst, woT_s, sem_a)
    for p in range(NP):
        for cp in pair_copies(p, b_src, b_dst, bwoT_h, bwoT_s, sem_b):
            cp.start()
        if p + 1 < NP:
            for cp in pair_copies(p + 1, a_src, a_dst, woT_h, woT_s, sem_a):
                cp.start()
    for cp in misc[2:]:
        cp.start()

    def half(u, e):
        sh = (16 * (1 - e)).astype(U32) if not isinstance(e, int) else jnp.uint32(16 * (1 - e))
        return pltpu.bitcast((u << sh) & jnp.uint32(0xFFFF0000), F32)

    def prep_a(h):
        p, e = h // 2, h % 2
        wq_s[e] = half(wq_r[p], e).astype(BF16)
        wkv_s[e, :, 0:DH] = half(wuk_r[p], e).astype(BF16)
        wkv_s[e, :, DH:2 * DH] = half(wuv_r[p], e).astype(BF16)

    def prep_b(h):
        p, e = h // 2, h % 2
        for j, w_ref in enumerate(b_dst):
            col = j * H * DH + h * DH
            col = col if isinstance(h, int) else pl.multiple_of(col, DH)
            bw_s[:, pl.ds(col, DH)] = half(w_ref[p], e).astype(BF16)
        row = h * DH if isinstance(h, int) else pl.multiple_of(h * DH, DH)
        bwo_s[pl.ds(row, DH), :] = bwoT_s[h].T

    def proj(h, r, RB):
        e = h % 2
        rows = pl.ds(r * RB, RB)
        q = jnp.dot(xa_s[rows, :], wq_s[e], preferred_element_type=F32)
        q_s[e, rows, :] = (q * QSCALE).astype(BF16)
        kv = jnp.dot(ckv_s[rows, :], wkv_s[e], preferred_element_type=F32)
        k_s[e, rows, :] = kv[:, 0:DH].astype(BF16)
        v_s[e, rows, :] = kv[:, DH:2 * DH].astype(BF16)

    def qk(e, i, k0, w):
        q = q_s[e, pl.ds(i * BQ, BQ), :]
        s = lax.dot_general(q, k_s[e, pl.ds(k0, w), :], NT, preferred_element_type=F32)
        if k0 + w > i * BQ:
            row = lax.broadcasted_iota(jnp.int32, (BQ, w), 0) + i * BQ
            col = lax.broadcasted_iota(jnp.int32, (BQ, w), 1) + k0
            s = jnp.where(col <= row, s, NEG)
        return s

    def upd(e, st, k0, w, s):
        mb = jnp.max(s, axis=1, keepdims=True)
        v = v_s[e, pl.ds(k0, w), :]
        if st is None:
            m = mb
            p = jnp.exp2(s - m)
            l = jnp.sum(p, axis=1, keepdims=True)
            acc = jnp.dot(p.astype(BF16), v, preferred_element_type=F32)
        else:
            m0, l0, a0 = st
            m = jnp.maximum(m0, mb)
            a = jnp.exp2(m0 - m)
            p = jnp.exp2(s - m)
            l = a * l0 + jnp.sum(p, axis=1, keepdims=True)
            acc = a * a0 + jnp.dot(p.astype(BF16), v, preferred_element_type=F32)
        return m, l, acc

    def att(h, filler):
        e = h % 2
        flat = []
        for i in range(S // BQ):
            kend = (i + 1) * BQ
            flat += [(i, k0, min(BK, kend - k0), k0 + BK >= kend) for k0 in range(0, kend, BK)]
        wo = woT_s[h]
        st = None
        pend = []

        def retire(st):
            i, k0, w, last, s = pend.pop(0)
            st = upd(e, st, k0, w, s)
            if last:
                _, l, acc = st
                ctx = (acc / l).astype(BF16)
                acc_s[pl.ds(i * BQ, BQ), :] += lax.dot_general(ctx, wo, NT, preferred_element_type=F32)
                filler(i)
                st = None
            return st

        for (i, k0, w, last) in flat:
            pend.append((i, k0, w, last, qk(e, i, k0, w)))
            if len(pend) > 1:
                st = retire(st)
        while pend:
            st = retire(st)

    NB = S // BQ
    prep_a(0)
    for r in range(NB):
        proj(0, r, BQ)

    def head(h, carry):
        @pl.when(h % 2 == 1)
        def _():
            pair_wait((h + 1) // 2, a_dst, woT_s, sem_a)

        @pl.when(h % 2 == 0)
        def _():
            pair_wait(h // 2, b_dst, bwoT_s, sem_b)

        prep_a(h + 1)
        prep_b(h)
        att(h, lambda i: proj(h + 1, i, BQ))
        return carry

    with jax.named_scope('Aloop'):
        lax.fori_loop(0, H - 1, head, 0)
    misc[2].wait()
    misc[3].wait()

    def last_fill(i):
        xb_s[pl.ds(i * 256, 256), :] = xT_s[1, :, pl.ds(i * 256, 256)].T
        if i == 0:
            prep_b(H - 1)
        rows = pl.ds(i * BQ, BQ)
        out_s[rows, 0:DM] = acc_s[rows, :].astype(BF16)

    att(H - 1, last_fill)

    L = NMEM + seg
    ri = lax.broadcasted_iota(jnp.int32, (L, L), 0)
    ci = lax.broadcasted_iota(jnp.int32, (L, L), 1)
    mask = (ri < NMEM) | (ri >= ci)

    def step(t, mem):
        rows = pl.ds(pl.multiple_of(t * seg, seg), seg)
        hcat = jnp.concatenate([mem, xb_s[rows, :].astype(F32)], axis=0)
        qkv_s[...] = lax.dot_general(hcat, bw_s[...], NN, preferred_element_type=F32)
        for hh in range(H):
            q = (qkv_s[:, pl.ds(hh * DH, DH)] * QSCALE).astype(BF16).astype(F32)
            k = qkv_s[:, pl.ds(H * DH + hh * DH, DH)].astype(BF16).astype(F32)
            v = qkv_s[:, pl.ds(2 * H * DH + hh * DH, DH)].astype(BF16).astype(F32)
            s = lax.dot_general(q, k, NT, preferred_element_type=F32)
            s = jnp.where(mask, s, NEG)
            m = jnp.max(s, axis=1, keepdims=True)
            p = jnp.exp2(s - m)
            l = jnp.sum(p, axis=1, keepdims=True)
            o = jnp.dot(p.astype(BF16).astype(F32), v, preferred_element_type=F32) / l
            ob_s[:, pl.ds(hh * DH, DH)] = o.astype(BF16).astype(F32)
        out = lax.dot_general(ob_s[...], bwo_s[...], NN, preferred_element_type=F32)
        out = out.astype(BF16)
        out_s[rows, DM:2 * DM] = out[NMEM:, :]

        @pl.when(t % OC == OC - 1)
        def _():
            out_copy(t // OC).start()
        return out[:NMEM, :].astype(F32)

    OC = 4

    def out_copy(c):
        rows = pl.ds(pl.multiple_of(c * (OC * seg), OC * seg), OC * seg)
        return pltpu.make_async_copy(out_s.at[rows, :], o_h.at[rows, :], sem_o.at[c])

    with jax.named_scope('Bloop'):
        lax.fori_loop(0, S // seg, step, mem0_s[...].astype(F32))
    for c in range(S // seg // OC):
        out_copy(c).wait()


@functools.partial(jax.jit, static_argnames=("B_seg_len",))
def pallas_concat_heads__compressed_kv_cla__memory_aug_recurrent_mem_tr__prompt_kernel(
        A_x, A_c_kv, A_w_q, A_w_uk, A_w_uv, A_w_o,
        B_x, B_mem0, B_Wq, B_Wk, B_Wv, B_Wo, B_seg_len):
    seg = int(B_seg_len)
    L = NMEM + seg
    vm = pl.BlockSpec(memory_space=pltpu.VMEM)
    hbm = pl.BlockSpec(memory_space=pl.ANY)
    NP = H // 2
    out = pl.pallas_call(
        functools.partial(_kernel, seg=seg),
        out_shape=jax.ShapeDtypeStruct((S, 2 * DM), BF16),
        in_specs=[hbm] * 12,
        out_specs=hbm,
        scratch_shapes=[
            pltpu.VMEM((2, DM, S), BF16),
            pltpu.VMEM((S, DM), BF16),
            pltpu.VMEM((S, DM), BF16),
            pltpu.VMEM((S, DC), BF16),
            pltpu.VMEM((H, DM, DH), BF16),
            pltpu.VMEM((H, DM, DH), BF16),
            pltpu.VMEM((NMEM, DM), BF16),
            pltpu.VMEM((NP, DM, DH), U32),
            pltpu.VMEM((NP, DC, DH), U32),
            pltpu.VMEM((NP, DC, DH), U32),
            pltpu.VMEM((NP, DM, DH), U32),
            pltpu.VMEM((NP, DM, DH), U32),
            pltpu.VMEM((NP, DM, DH), U32),
            pltpu.VMEM((2, DM, DH), BF16),
            pltpu.VMEM((2, DC, 2 * DH), BF16),
            pltpu.VMEM((2, S, DH), BF16),
            pltpu.VMEM((2, S, DH), BF16),
            pltpu.VMEM((2, S, DH), BF16),
            pltpu.VMEM((S, DM), F32),
            pltpu.VMEM((DM, 3 * H * DH), BF16),
            pltpu.VMEM((H * DH, DM), BF16),
            pltpu.VMEM((L, 3 * H * DH), F32),
            pltpu.VMEM((L, H * DH), F32),
            pltpu.VMEM((S, 2 * DM), BF16),
            pltpu.SemaphoreType.DMA((NP,)),
            pltpu.SemaphoreType.DMA((NP,)),
            pltpu.SemaphoreType.DMA((4,)),
            pltpu.SemaphoreType.DMA((S // seg // 4,)),
        ],
        compiler_params=pltpu.CompilerParams(vmem_limit_bytes=124 * 2 ** 20),
    )(jnp.swapaxes(A_x, 1, 2).reshape(DM, S), A_c_kv.reshape(S, DC),
      A_w_q, A_w_uk, A_w_uv, jnp.swapaxes(A_w_o, 1, 2),
      jnp.swapaxes(B_x, 1, 2).reshape(DM, S), B_mem0.reshape(NMEM, DM),
      B_Wq, B_Wk, B_Wv, jnp.swapaxes(B_Wo, 1, 2))
    return out.reshape(1, S, 2 * DM)
```

```python
import functools

import jax
import jax.numpy as jnp
from jax import lax
from jax.experimental import pallas as pl
from jax.experimental.pallas import tpu as pltpu

F32 = jnp.float32
BF16 = jnp.bfloat16
U32 = jnp.uint32
LOG2E = 1.4426950408889634
NEG = -1e30

S = 2048
DM = 576
DC = 512
H = 32
DH = 128
NMEM = 8
BQ = 256
BK = 512
G = 8
HG = H // G
GW = 3 * HG * DH
NT = (((1,), (1,)), ((), ()))
NN = (((1,), (0,)), ((), ()))
QSCALE = DH ** -0.5 * LOG2E


def _split(u):
    lo = pltpu.bitcast(u << 16, F32)
    hi = pltpu.bitcast(u & jnp.uint32(0xFFFF0000), F32)
    return lo, hi


def _r16(a):
    return a.astype(BF16).astype(F32)


def _kernel(xaT_h, ckv_h, wq_h, wuk_h, wuv_h, woT_h,
            xbT_h, mem0_h, bwq_h, bwk_h, bwv_h, bwoT_h,
            o_h,
            xT_s, xa_s, xb_s, ckv_s, woT_s, bwoT_s, mem0_s,
            wq_r, wuk_r, wuv_r, bwq_r, bwk_r, bwv_r,
            wq_s, wkv_s, q_s, k_s, v_s, acc_s,
            bw_s, bwo_s, qkv_s, ob_s, out_s,
            sem_a, sem_b, sem_m, sem_o, *, seg):
    NP = H // 2
    misc = [pltpu.make_async_copy(xaT_h, xT_s.at[0], sem_m.at[0]),
            pltpu.make_async_copy(ckv_h, ckv_s, sem_m.at[1]),
            pltpu.make_async_copy(xbT_h, xT_s.at[1], sem_m.at[2]),
            pltpu.make_async_copy(mem0_h, mem0_s, sem_m.at[3])]

    def pair_copies(p, srcs, dsts, oT_h, oT_s, sem):
        cps = [pltpu.make_async_copy(s_.bitcast(U32).at[:, p, :], d_.at[p], sem.at[p])
               for s_, d_ in zip(srcs, dsts)]
        cps.append(pltpu.make_async_copy(oT_h.at[pl.ds(2 * p, 2)], oT_s.at[pl.ds(2 * p, 2)], sem.at[p]))
        return cps

    def pair_wait(p, dsts, oT_s, sem):
        for d_ in dsts:
            pltpu.make_async_copy(d_.at[p], d_.at[p], sem.at[p]).wait()
        sl = oT_s.at[pl.ds(2 * p, 2)]
        pltpu.make_async_copy(sl, sl, sem.at[p]).wait()

    a_src, a_dst = (wq_h, wuk_h, wuv_h), (wq_r, wuk_r, wuv_r)
    b_src, b_dst = (bwq_h, bwk_h, bwv_h), (bwq_r, bwk_r, bwv_r)
    misc[0].start()
    misc[1].start()
    for cp in pair_copies(0, a_src, a_dst, woT_h, woT_s, sem_a):
        cp.start()
    acc_s[...] = jnp.zeros_like(acc_s)
    misc[0].wait()
    for r in range(S // 256):
        xa_s[pl.ds(r * 256, 256), :] = xT_s[0, :, pl.ds(r * 256, 256)].T
    misc[1].wait()
    pair_wait(0, a_dst, woT_s, sem_a)
    for cp in pair_copies(1, a_src, a_dst, woT_h, woT_s, sem_a):
        cp.start()
    for cp in pair_copies(0, b_src, b_dst, bwoT_h, bwoT_s, sem_b):
        cp.start()
    for cp in pair_copies(2, a_src, a_dst, woT_h, woT_s, sem_a):
        cp.start()
    for cp in pair_copies(1, b_src, b_dst, bwoT_h, bwoT_s, sem_b):
        cp.start()

    def half(u, e):
        sh = (16 * (1 - e)).astype(U32) if not isinstance(e, int) else jnp.uint32(16 * (1 - e))
        return pltpu.bitcast((u << sh) & jnp.uint32(0xFFFF0000), F32)

    def prep_a(h):
        p, e = h // 2, h % 2
        wq_s[e] = half(wq_r[p], e).astype(BF16)
        wkv_s[e, :, 0:DH] = half(wuk_r[p], e).astype(BF16)
        wkv_s[e, :, DH:2 * DH] = half(wuv_r[p], e).astype(BF16)

    def prep_b(h):
        p, e = h // 2, h % 2
        for j, w_ref in enumerate(b_dst):
            col = (h // HG) * GW + (j * HG + h % HG) * DH
            col = col if isinstance(h, int) else pl.multiple_of(col, DH)
            bw_s[:, pl.ds(col, DH)] = half(w_ref[p], e).astype(BF16)
        row = h * DH if isinstance(h, int) else pl.multiple_of(h * DH, DH)
        bwo_s[pl.ds(row, DH), :] = bwoT_s[h].T

    def proj(h, r, RB):
        e = h % 2
        rows = pl.ds(r * RB, RB)
        q = jnp.dot(xa_s[rows, :], wq_s[e], preferred_element_type=F32)
        q_s[e, rows, :] = (q * QSCALE).astype(BF16)
        kv = jnp.dot(ckv_s[rows, :], wkv_s[e], preferred_element_type=F32)
        k_s[e, rows, :] = kv[:, 0:DH].astype(BF16)
        v_s[e, rows, :] = kv[:, DH:2 * DH].astype(BF16)

    def qk(e, i, k0, w):
        q = q_s[e, pl.ds(i * BQ, BQ), :]
        s = lax.dot_general(q, k_s[e, pl.ds(k0, w), :], NT, preferred_element_type=F32)
        if k0 + w > i * BQ:
            row = lax.broadcasted_iota(jnp.int32, (BQ, w), 0) + i * BQ
            col = lax.broadcasted_iota(jnp.int32, (BQ, w), 1) + k0
            s = jnp.where(col <= row, s, NEG)
        return s

    def upd(e, st, k0, w, s):
        mb = jnp.max(s, axis=1, keepdims=True)
        v = v_s[e, pl.ds(k0, w), :]
        if st is None:
            m = mb
            p = jnp.exp2(s - m)
            l = jnp.sum(p, axis=1, keepdims=True)
            acc = jnp.dot(p.astype(BF16), v, preferred_element_type=F32)
        else:
            m0, l0, a0 = st
            m = jnp.maximum(m0, mb)
            a = jnp.exp2(m0 - m)
            p = jnp.exp2(s - m)
            l = a * l0 + jnp.sum(p, axis=1, keepdims=True)
            acc = a * a0 + jnp.dot(p.astype(BF16), v, preferred_element_type=F32)
        return m, l, acc

    def att(h, filler):
        e = h % 2
        flat = []
        for i in range(S // BQ):
            kend = (i + 1) * BQ
            flat += [(i, k0, min(BK, kend - k0), k0 + BK >= kend) for k0 in range(0, kend, BK)]
        st = None
        pend = []

        def retire(st):
            i, k0, w, last, s = pend.pop(0)
            st = upd(e, st, k0, w, s)
            if last:
                _, l, acc = st
                ctx = (acc / l).astype(BF16)
                acc_s[pl.ds(i * BQ, BQ), :] += lax.dot_general(ctx, woT_s[h], NT, preferred_element_type=F32)
                filler(i)
                st = None
            return st

        for (i, k0, w, last) in flat:
            pend.append((i, k0, w, last, qk(e, i, k0, w)))
            if len(pend) > 1:
                st = retire(st)
        while pend:
            st = retire(st)

    NB = S // BQ
    prep_a(0)
    for r in range(NB):
        proj(0, r, BQ)

    def head(h, carry):
        @pl.when(h % 2 == 1)
        def _():
            pair_wait((h + 1) // 2, a_dst, woT_s, sem_a)

        @pl.when((h % 2 == 1) & (h < H - 5))
        def _():
            for cp in pair_copies((h + 5) // 2, a_src, a_dst, woT_h, woT_s, sem_a):
                cp.start()

        @pl.when((h % 2 == 0) & (h < H - 4))
        def _():
            for cp in pair_copies(h // 2 + 2, b_src, b_dst, bwoT_h, bwoT_s, sem_b):
                cp.start()

        @pl.when(h == H - 4)
        def _():
            for cp in misc[2:]:
                cp.start()

        @pl.when(h % 2 == 0)
        def _():
            pair_wait(h // 2, b_dst, bwoT_s, sem_b)

        prep_a(h + 1)
        prep_b(h)
        att(h, lambda i: proj(h + 1, i, BQ))
        return carry

    with jax.named_scope('Aloop'):
        lax.fori_loop(0, H - 1, head, 0)
    misc[2].wait()
    misc[3].wait()

    def last_fill(i):
        xb_s[pl.ds(i * 256, 256), :] = xT_s[1, :, pl.ds(i * 256, 256)].T
        if i == 0:
            prep_b(H - 1)
        rows = pl.ds(i * BQ, BQ)
        out_s[rows, 0:DM] = acc_s[rows, :].astype(BF16)

    att(H - 1, last_fill)

    L = NMEM + seg
    ri = lax.broadcasted_iota(jnp.int32, (L, L), 0)
    ci = lax.broadcasted_iota(jnp.int32, (L, L), 1)
    mask = (ri < NMEM) | (ri >= ci)

    def step(t, mem):
        rows = pl.ds(pl.multiple_of(t * seg, seg), seg)
        hcat = jnp.concatenate([mem, xb_s[rows, :].astype(F32)], axis=0)

        def pj(g):
            cols = pl.ds(g * GW, GW)
            qkv_s[:, cols] = lax.dot_general(hcat, bw_s[:, cols], NN, preferred_element_type=F32)

        def at(g):
            for j in range(HG):
                q = _r16(qkv_s[:, pl.ds(g * GW + j * DH, DH)] * QSCALE)
                k = _r16(qkv_s[:, pl.ds(g * GW + (HG + j) * DH, DH)])
                v = _r16(qkv_s[:, pl.ds(g * GW + (2 * HG + j) * DH, DH)])
                s = lax.dot_general(q, k, NT, preferred_element_type=F32)
                s = jnp.where(mask, s, NEG)
                m = jnp.max(s, axis=1, keepdims=True)
                p = jnp.exp2(s - m)
                l = jnp.sum(p, axis=1, keepdims=True)
                o = jnp.dot(_r16(p), v, preferred_element_type=F32) / l
                ob_s[:, pl.ds((g * HG + j) * DH, DH)] = _r16(o)

        def op(g):
            sl = pl.ds(g * HG * DH, HG * DH)
            return lax.dot_general(ob_s[:, sl], bwo_s[sl, :], NN, preferred_element_type=F32)

        out = None
        for g in range(G + 2):
            if g < G:
                pj(g)
            if 0 <= g - 1 < G:
                at(g - 1)
            if 0 <= g - 2 < G:
                r = op(g - 2)
                out = r if out is None else out + r
        out = out.astype(BF16)
        out_s[rows, DM:2 * DM] = out[NMEM:, :]

        @pl.when(t % OC == OC - 1)
        def _():
            out_copy(t // OC).start()
        return out[:NMEM, :].astype(F32)

    OC = 4

    def out_copy(c):
        rows = pl.ds(pl.multiple_of(c * (OC * seg), OC * seg), OC * seg)
        return pltpu.make_async_copy(out_s.at[rows, :], o_h.at[rows, :], sem_o.at[c])

    with jax.named_scope('Bloop'):
        lax.fori_loop(0, S // seg, step, mem0_s[...].astype(F32))
    for c in range(S // seg // OC):
        out_copy(c).wait()


@functools.partial(jax.jit, static_argnames=("B_seg_len",))
def pallas_concat_heads__compressed_kv_cla__memory_aug_recurrent_mem_tr__prompt_kernel(
        A_x, A_c_kv, A_w_q, A_w_uk, A_w_uv, A_w_o,
        B_x, B_mem0, B_Wq, B_Wk, B_Wv, B_Wo, B_seg_len):
    seg = int(B_seg_len)
    L = NMEM + seg
    vm = pl.BlockSpec(memory_space=pltpu.VMEM)
    hbm = pl.BlockSpec(memory_space=pl.ANY)
    NP = H // 2
    out = pl.pallas_call(
        functools.partial(_kernel, seg=seg),
        out_shape=jax.ShapeDtypeStruct((S, 2 * DM), BF16),
        in_specs=[hbm] * 12,
        out_specs=hbm,
        scratch_shapes=[
            pltpu.VMEM((2, DM, S), BF16),
            pltpu.VMEM((S, DM), BF16),
            pltpu.VMEM((S, DM), BF16),
            pltpu.VMEM((S, DC), BF16),
            pltpu.VMEM((H, DM, DH), BF16),
            pltpu.VMEM((H, DM, DH), BF16),
            pltpu.VMEM((NMEM, DM), BF16),
            pltpu.VMEM((NP, DM, DH), U32),
            pltpu.VMEM((NP, DC, DH), U32),
            pltpu.VMEM((NP, DC, DH), U32),
            pltpu.VMEM((NP, DM, DH), U32),
            pltpu.VMEM((NP, DM, DH), U32),
            pltpu.VMEM((NP, DM, DH), U32),
            pltpu.VMEM((2, DM, DH), BF16),
            pltpu.VMEM((2, DC, 2 * DH), BF16),
            pltpu.VMEM((2, S, DH), BF16),
            pltpu.VMEM((2, S, DH), BF16),
            pltpu.VMEM((2, S, DH), BF16),
            pltpu.VMEM((S, DM), F32),
            pltpu.VMEM((DM, 3 * H * DH), BF16),
            pltpu.VMEM((H * DH, DM), BF16),
            pltpu.VMEM((L, 3 * H * DH), F32),
            pltpu.VMEM((L, H * DH), F32),
            pltpu.VMEM((S, 2 * DM), BF16),
            pltpu.SemaphoreType.DMA((NP,)),
            pltpu.SemaphoreType.DMA((NP,)),
            pltpu.SemaphoreType.DMA((4,)),
            pltpu.SemaphoreType.DMA((S // seg // 4,)),
        ],
        compiler_params=pltpu.CompilerParams(vmem_limit_bytes=124 * 2 ** 20),
    )(jnp.swapaxes(A_x, 1, 2).reshape(DM, S), A_c_kv.reshape(S, DC),
      A_w_q, A_w_uk, A_w_uv, jnp.swapaxes(A_w_o, 1, 2),
      jnp.swapaxes(B_x, 1, 2).reshape(DM, S), B_mem0.reshape(NMEM, DM),
      B_Wq, B_Wk, B_Wv, jnp.swapaxes(B_Wo, 1, 2))
    return out.reshape(1, S, 2 * DM)
```

```python
import functools

import jax
import jax.numpy as jnp
from jax import lax
from jax.experimental import pallas as pl
from jax.experimental.pallas import tpu as pltpu

F32 = jnp.float32
BF16 = jnp.bfloat16
U32 = jnp.uint32
LOG2E = 1.4426950408889634
NEG = -1e30

S = 2048
DM = 576
DC = 512
H = 32
DH = 128
NMEM = 8
BQ = 256
BK = 512
G = 8
HG = H // G
GW = 3 * HG * DH
NT = (((1,), (1,)), ((), ()))
NN = (((1,), (0,)), ((), ()))
QSCALE = DH ** -0.5 * LOG2E


def _split(u):
    lo = pltpu.bitcast(u << 16, F32)
    hi = pltpu.bitcast(u & jnp.uint32(0xFFFF0000), F32)
    return lo, hi


def _r16(a):
    return a.astype(BF16).astype(F32)


def _kernel(xaT_h, ckv_h, wq_h, wuk_h, wuv_h, woT_h,
            xbT_h, mem0_h, bwq_h, bwk_h, bwv_h, bwoT_h,
            o_h,
            xT_s, xa_s, xb_s, ckv_s, woT_s, bwoT_s, mem0_s,
            wq_r, wuk_r, wuv_r, bwq_r, bwk_r, bwv_r,
            wq_s, wkv_s, q_s, k_s, v_s, acc_s,
            bw_s, bwo_s, qkv_s, ob_s, out_s,
            sem_a, sem_b, sem_m, sem_o, *, seg):
    NP = H // 2
    misc = [pltpu.make_async_copy(xaT_h, xT_s.at[0], sem_m.at[0]),
            pltpu.make_async_copy(ckv_h, ckv_s, sem_m.at[1]),
            pltpu.make_async_copy(xbT_h, xT_s.at[1], sem_m.at[2]),
            pltpu.make_async_copy(mem0_h, mem0_s, sem_m.at[3])]

    def pair_copies(p, srcs, dsts, oT_h, oT_s, sem):
        cps = [pltpu.make_async_copy(s_.bitcast(U32).at[:, p, :], d_.at[p], sem.at[p])
               for s_, d_ in zip(srcs, dsts)]
        cps.append(pltpu.make_async_copy(oT_h.at[pl.ds(2 * p, 2)], oT_s.at[pl.ds(2 * p, 2)], sem.at[p]))
        return cps

    def pair_wait(p, dsts, oT_s, sem):
        for d_ in dsts:
            pltpu.make_async_copy(d_.at[p], d_.at[p], sem.at[p]).wait()
        sl = oT_s.at[pl.ds(2 * p, 2)]
        pltpu.make_async_copy(sl, sl, sem.at[p]).wait()

    a_src, a_dst = (wq_h, wuk_h, wuv_h), (wq_r, wuk_r, wuv_r)
    b_src, b_dst = (bwq_h, bwk_h, bwv_h), (bwq_r, bwk_r, bwv_r)
    misc[0].start()
    misc[1].start()
    for cp in pair_copies(0, a_src, a_dst, woT_h, woT_s, sem_a):
        cp.start()
    acc_s[...] = jnp.zeros_like(acc_s)
    misc[0].wait()
    for r in range(S // 256):
        xa_s[pl.ds(r * 256, 256), :] = xT_s[0, :, pl.ds(r * 256, 256)].T
    misc[1].wait()
    pair_wait(0, a_dst, woT_s, sem_a)
    for cp in pair_copies(1, a_src, a_dst, woT_h, woT_s, sem_a):
        cp.start()
    for cp in pair_copies(0, b_src, b_dst, bwoT_h, bwoT_s, sem_b):
        cp.start()
    for cp in pair_copies(2, a_src, a_dst, woT_h, woT_s, sem_a):
        cp.start()
    for cp in pair_copies(1, b_src, b_dst, bwoT_h, bwoT_s, sem_b):
        cp.start()

    def half(u, e):
        sh = (16 * (1 - e)).astype(U32) if not isinstance(e, int) else jnp.uint32(16 * (1 - e))
        return pltpu.bitcast((u << sh) & jnp.uint32(0xFFFF0000), F32)

    def prep_a(h, p, e):
        wq_s[e] = half(wq_r[p], e).astype(BF16)
        wkv_s[e, :, 0:DH] = half(wuk_r[p], e).astype(BF16)
        wkv_s[e, :, DH:2 * DH] = half(wuv_r[p], e).astype(BF16)

    def prep_b(h, p, e):
        for j, w_ref in enumerate(b_dst):
            col = (h // HG) * GW + (j * HG + h % HG) * DH
            col = col if isinstance(h, int) else pl.multiple_of(col, DH)
            bw_s[:, pl.ds(col, DH)] = half(w_ref[p], e).astype(BF16)
        row = h * DH if isinstance(h, int) else pl.multiple_of(h * DH, DH)
        bwo_s[pl.ds(row, DH), :] = bwoT_s[h].T

    def proj(h, r, RB):
        e = h % 2
        rows = pl.ds(r * RB, RB)
        q = jnp.dot(xa_s[rows, :], wq_s[e], preferred_element_type=F32)
        q_s[e, rows, :] = (q * QSCALE).astype(BF16)
        kv = jnp.dot(ckv_s[rows, :], wkv_s[e], preferred_element_type=F32)
        k_s[e, rows, :] = kv[:, 0:DH].astype(BF16)
        v_s[e, rows, :] = kv[:, DH:2 * DH].astype(BF16)

    def qk(e, i, k0, w):
        q = q_s[e, pl.ds(i * BQ, BQ), :]
        s = lax.dot_general(q, k_s[e, pl.ds(k0, w), :], NT, preferred_element_type=F32)
        if k0 + w > i * BQ:
            row = lax.broadcasted_iota(jnp.int32, (BQ, w), 0) + i * BQ
            col = lax.broadcasted_iota(jnp.int32, (BQ, w), 1) + k0
            s = jnp.where(col <= row, s, NEG)
        return s

    def upd(e, st, k0, w, s):
        mb = jnp.max(s, axis=1, keepdims=True)
        v = v_s[e, pl.ds(k0, w), :]
        if st is None:
            m = mb
            p = jnp.exp2(s - m)
            l = jnp.sum(p, axis=1, keepdims=True)
            acc = jnp.dot(p.astype(BF16), v, preferred_element_type=F32)
        else:
            m0, l0, a0 = st
            m = jnp.maximum(m0, mb)
            a = jnp.exp2(m0 - m)
            p = jnp.exp2(s - m)
            l = a * l0 + jnp.sum(p, axis=1, keepdims=True)
            acc = a * a0 + jnp.dot(p.astype(BF16), v, preferred_element_type=F32)
        return m, l, acc

    def att(h, e, filler):
        flat = []
        for i in range(S // BQ):
            kend = (i + 1) * BQ
            flat += [(i, k0, min(BK, kend - k0), k0 + BK >= kend) for k0 in range(0, kend, BK)]
        st = None
        pend = []

        def retire(st):
            i, k0, w, last, s = pend.pop(0)
            st = upd(e, st, k0, w, s)
            if last:
                _, l, acc = st
                ctx = (acc / l).astype(BF16)
                acc_s[pl.ds(i * BQ, BQ), :] += lax.dot_general(ctx, woT_s[h], NT, preferred_element_type=F32)
                filler(i)
                st = None
            return st

        for (i, k0, w, last) in flat:
            pend.append((i, k0, w, last, qk(e, i, k0, w)))
            if len(pend) > 1:
                st = retire(st)
        while pend:
            st = retire(st)

    NB = S // BQ
    prep_a(0, 0, 0)
    for r in range(NB):
        proj(0, r, BQ)

    def pair(p, carry):
        pair_wait(p, b_dst, bwoT_s, sem_b)

        @pl.when(p < NP - 2)
        def _():
            for cp in pair_copies(p + 2, b_src, b_dst, bwoT_h, bwoT_s, sem_b):
                cp.start()

        @pl.when(p < NP - 3)
        def _():
            for cp in pair_copies(p + 3, a_src, a_dst, woT_h, woT_s, sem_a):
                cp.start()

        @pl.when(p == NP - 2)
        def _():
            for cp in misc[2:]:
                cp.start()

        h = 2 * p
        prep_a(h + 1, p, 1)
        prep_b(h, p, 0)
        att(h, 0, lambda i: proj(1, i, BQ))
        pair_wait(p + 1, a_dst, woT_s, sem_a)
        prep_a(h + 2, p + 1, 0)
        prep_b(h + 1, p, 1)
        att(h + 1, 1, lambda i: proj(0, i, BQ))
        return carry

    with jax.named_scope('Aloop'):
        lax.fori_loop(0, NP - 1, pair, 0)
    pair_wait(NP - 1, b_dst, bwoT_s, sem_b)
    prep_a(H - 1, NP - 1, 1)
    prep_b(H - 2, NP - 1, 0)
    att(H - 2, 0, lambda i: proj(1, i, BQ))
    misc[2].wait()
    misc[3].wait()

    def last_fill(i):
        xb_s[pl.ds(i * 256, 256), :] = xT_s[1, :, pl.ds(i * 256, 256)].T
        if i == 0:
            prep_b(H - 1, NP - 1, 1)
        rows = pl.ds(i * BQ, BQ)
        out_s[rows, 0:DM] = acc_s[rows, :].astype(BF16)

    att(H - 1, 1, last_fill)

    L = NMEM + seg
    ri = lax.broadcasted_iota(jnp.int32, (L, L), 0)
    ci = lax.broadcasted_iota(jnp.int32, (L, L), 1)
    mask = (ri < NMEM) | (ri >= ci)

    def step(t, mem):
        rows = pl.ds(pl.multiple_of(t * seg, seg), seg)
        hcat = jnp.concatenate([mem, xb_s[rows, :].astype(F32)], axis=0)

        def pj(g):
            cols = pl.ds(g * GW, GW)
            qkv_s[:, cols] = lax.dot_general(hcat, bw_s[:, cols], NN, preferred_element_type=F32)

        def at(g):
            for j in range(HG):
                q = _r16(qkv_s[:, pl.ds(g * GW + j * DH, DH)] * QSCALE)
                k = _r16(qkv_s[:, pl.ds(g * GW + (HG + j) * DH, DH)])
                v = _r16(qkv_s[:, pl.ds(g * GW + (2 * HG + j) * DH, DH)])
                s = lax.dot_general(q, k, NT, preferred_element_type=F32)
                s = jnp.where(mask, s, NEG)
                m = jnp.max(s, axis=1, keepdims=True)
                p = jnp.exp2(s - m)
                l = jnp.sum(p, axis=1, keepdims=True)
                o = jnp.dot(_r16(p), v, preferred_element_type=F32) / l
                ob_s[:, pl.ds((g * HG + j) * DH, DH)] = _r16(o)

        def op(g):
            sl = pl.ds(g * HG * DH, HG * DH)
            return lax.dot_general(ob_s[:, sl], bwo_s[sl, :], NN, preferred_element_type=F32)

        out = None
        for g in range(G + 2):
            if g < G:
                pj(g)
            if 0 <= g - 1 < G:
                at(g - 1)
            if 0 <= g - 2 < G:
                r = op(g - 2)
                out = r if out is None else out + r
        out = out.astype(BF16)
        out_s[rows, DM:2 * DM] = out[NMEM:, :]

        @pl.when(t % OC == OC - 1)
        def _():
            out_copy(t // OC).start()
        return out[:NMEM, :].astype(F32)

    OC = 4

    def out_copy(c):
        rows = pl.ds(pl.multiple_of(c * (OC * seg), OC * seg), OC * seg)
        return pltpu.make_async_copy(out_s.at[rows, :], o_h.at[rows, :], sem_o.at[c])

    with jax.named_scope('Bloop'):
        lax.fori_loop(0, S // seg, step, mem0_s[...].astype(F32))
    for c in range(S // seg // OC):
        out_copy(c).wait()


@functools.partial(jax.jit, static_argnames=("B_seg_len",))
def pallas_concat_heads__compressed_kv_cla__memory_aug_recurrent_mem_tr__prompt_kernel(
        A_x, A_c_kv, A_w_q, A_w_uk, A_w_uv, A_w_o,
        B_x, B_mem0, B_Wq, B_Wk, B_Wv, B_Wo, B_seg_len):
    seg = int(B_seg_len)
    L = NMEM + seg
    vm = pl.BlockSpec(memory_space=pltpu.VMEM)
    hbm = pl.BlockSpec(memory_space=pl.ANY)
    NP = H // 2
    out = pl.pallas_call(
        functools.partial(_kernel, seg=seg),
        out_shape=jax.ShapeDtypeStruct((S, 2 * DM), BF16),
        in_specs=[hbm] * 12,
        out_specs=hbm,
        scratch_shapes=[
            pltpu.VMEM((2, DM, S), BF16),
            pltpu.VMEM((S, DM), BF16),
            pltpu.VMEM((S, DM), BF16),
            pltpu.VMEM((S, DC), BF16),
            pltpu.VMEM((H, DM, DH), BF16),
            pltpu.VMEM((H, DM, DH), BF16),
            pltpu.VMEM((NMEM, DM), BF16),
            pltpu.VMEM((NP, DM, DH), U32),
            pltpu.VMEM((NP, DC, DH), U32),
            pltpu.VMEM((NP, DC, DH), U32),
            pltpu.VMEM((NP, DM, DH), U32),
            pltpu.VMEM((NP, DM, DH), U32),
            pltpu.VMEM((NP, DM, DH), U32),
            pltpu.VMEM((2, DM, DH), BF16),
            pltpu.VMEM((2, DC, 2 * DH), BF16),
            pltpu.VMEM((2, S, DH), BF16),
            pltpu.VMEM((2, S, DH), BF16),
            pltpu.VMEM((2, S, DH), BF16),
            pltpu.VMEM((S, DM), F32),
            pltpu.VMEM((DM, 3 * H * DH), BF16),
            pltpu.VMEM((H * DH, DM), BF16),
            pltpu.VMEM((L, 3 * H * DH), F32),
            pltpu.VMEM((L, H * DH), F32),
            pltpu.VMEM((S, 2 * DM), BF16),
            pltpu.SemaphoreType.DMA((NP,)),
            pltpu.SemaphoreType.DMA((NP,)),
            pltpu.SemaphoreType.DMA((4,)),
            pltpu.SemaphoreType.DMA((S // seg // 4,)),
        ],
        compiler_params=pltpu.CompilerParams(vmem_limit_bytes=124 * 2 ** 20),
    )(jnp.swapaxes(A_x, 1, 2).reshape(DM, S), A_c_kv.reshape(S, DC),
      A_w_q, A_w_uk, A_w_uv, jnp.swapaxes(A_w_o, 1, 2),
      jnp.swapaxes(B_x, 1, 2).reshape(DM, S), B_mem0.reshape(NMEM, DM),
      B_Wq, B_Wk, B_Wv, jnp.swapaxes(B_Wo, 1, 2))
    return out.reshape(1, S, 2 * DM)
```

```python
import functools

import jax
import jax.numpy as jnp
from jax import lax
from jax.experimental import pallas as pl
from jax.experimental.pallas import tpu as pltpu

F32 = jnp.float32
BF16 = jnp.bfloat16
U32 = jnp.uint32
LOG2E = 1.4426950408889634
NEG = -1e30

S = 2048
DM = 576
DC = 512
H = 32
DH = 128
NMEM = 8
BQ = 256
BK = 512
G = 8
HG = H // G
GW = 3 * HG * DH
NT = (((1,), (1,)), ((), ()))
NN = (((1,), (0,)), ((), ()))
QSCALE = DH ** -0.5 * LOG2E


def _split(u):
    lo = pltpu.bitcast(u << 16, F32)
    hi = pltpu.bitcast(u & jnp.uint32(0xFFFF0000), F32)
    return lo, hi


def _r16(a):
    return a.astype(BF16).astype(F32)


def _kernel(xaT_h, ckv_h, wq_h, wuk_h, wuv_h, woT_h,
            xbT_h, mem0_h, bwq_h, bwk_h, bwv_h, bwoT_h,
            o_h,
            xT_s, xa_s, xb_s, ckv_s, woT_s, bwoT_s, mem0_s,
            wq_r, wuk_r, wuv_r, bwq_r, bwk_r, bwv_r,
            wq_s, wkv_s, q_s, k_s, v_s, acc_s,
            bw_s, bwo_s, qkv_s, ob_s, out_s,
            sem_a, sem_b, sem_m, sem_o, *, seg):
    NP = H // 2
    misc = [pltpu.make_async_copy(xaT_h, xT_s.at[0], sem_m.at[0]),
            pltpu.make_async_copy(ckv_h, ckv_s, sem_m.at[1]),
            pltpu.make_async_copy(xbT_h, xT_s.at[1], sem_m.at[2]),
            pltpu.make_async_copy(mem0_h, mem0_s, sem_m.at[3])]

    def pair_copies(p, srcs, dsts, oT_h, oT_s, sem):
        cps = [pltpu.make_async_copy(s_.bitcast(U32).at[:, p, :], d_.at[p], sem.at[p])
               for s_, d_ in zip(srcs, dsts)]
        cps.append(pltpu.make_async_copy(oT_h.at[pl.ds(2 * p, 2)], oT_s.at[pl.ds(2 * p, 2)], sem.at[p]))
        return cps

    def pair_wait(p, dsts, oT_s, sem):
        for d_ in dsts:
            pltpu.make_async_copy(d_.at[p], d_.at[p], sem.at[p]).wait()
        sl = oT_s.at[pl.ds(2 * p, 2)]
        pltpu.make_async_copy(sl, sl, sem.at[p]).wait()

    a_src, a_dst = (wq_h, wuk_h, wuv_h), (wq_r, wuk_r, wuv_r)
    b_src, b_dst = (bwq_h, bwk_h, bwv_h), (bwq_r, bwk_r, bwv_r)
    misc[0].start()
    misc[1].start()
    for cp in pair_copies(0, a_src, a_dst, woT_h, woT_s, sem_a):
        cp.start()
    acc_s[...] = jnp.zeros_like(acc_s)
    misc[0].wait()
    for r in range(S // 256):
        xa_s[pl.ds(r * 256, 256), :] = xT_s[0, :, pl.ds(r * 256, 256)].T
    misc[1].wait()
    pair_wait(0, a_dst, woT_s, sem_a)
    for cp in pair_copies(1, a_src, a_dst, woT_h, woT_s, sem_a):
        cp.start()
    for cp in pair_copies(0, b_src, b_dst, bwoT_h, bwoT_s, sem_b):
        cp.start()
    for cp in pair_copies(2, a_src, a_dst, woT_h, woT_s, sem_a):
        cp.start()
    for cp in pair_copies(1, b_src, b_dst, bwoT_h, bwoT_s, sem_b):
        cp.start()

    def half(u, e):
        sh = (16 * (1 - e)).astype(U32) if not isinstance(e, int) else jnp.uint32(16 * (1 - e))
        return pltpu.bitcast((u << sh) & jnp.uint32(0xFFFF0000), F32)

    def prep_a(h, p, e):
        wq_s[e] = half(wq_r[p], e).astype(BF16)
        wkv_s[e, :, 0:DH] = half(wuk_r[p], e).astype(BF16)
        wkv_s[e, :, DH:2 * DH] = half(wuv_r[p], e).astype(BF16)

    def prep_b(h, p, e):
        for j, w_ref in enumerate(b_dst):
            col = (h // HG) * GW + (j * HG + h % HG) * DH
            col = col if isinstance(h, int) else pl.multiple_of(col, DH)
            bw_s[:, pl.ds(col, DH)] = half(w_ref[p], e).astype(BF16)
        row = h * DH if isinstance(h, int) else pl.multiple_of(h * DH, DH)
        bwo_s[pl.ds(row, DH), :] = bwoT_s[h].T

    def proj(h, r, RB):
        e = h % 2
        rows = pl.ds(r * RB, RB)
        q = jnp.dot(xa_s[rows, :], wq_s[e], preferred_element_type=F32)
        q_s[e, rows, :] = (q * QSCALE).astype(BF16)
        kv = jnp.dot(ckv_s[rows, :], wkv_s[e], preferred_element_type=F32)
        k_s[e, rows, :] = kv[:, 0:DH].astype(BF16)
        v_s[e, rows, :] = kv[:, DH:2 * DH].astype(BF16)

    def qk(e, i, k0, w):
        q = q_s[e, pl.ds(i * BQ, BQ), :]
        s = lax.dot_general(q, k_s[e, pl.ds(k0, w), :], NT, preferred_element_type=F32)
        if k0 + w > i * BQ:
            row = lax.broadcasted_iota(jnp.int32, (BQ, w), 0) + i * BQ
            col = lax.broadcasted_iota(jnp.int32, (BQ, w), 1) + k0
            s = jnp.where(col <= row, s, NEG)
        return s

    def upd(e, st, k0, w, s):
        mb = jnp.max(s, axis=1, keepdims=True)
        v = v_s[e, pl.ds(k0, w), :]
        if st is None:
            m = mb
            p = jnp.exp2(s - m)
            l = jnp.sum(p, axis=1, keepdims=True)
            acc = jnp.dot(p.astype(BF16), v, preferred_element_type=F32)
        else:
            m0, l0, a0 = st
            m = jnp.maximum(m0, mb)
            a = jnp.exp2(m0 - m)
            p = jnp.exp2(s - m)
            l = a * l0 + jnp.sum(p, axis=1, keepdims=True)
            acc = a * a0 + jnp.dot(p.astype(BF16), v, preferred_element_type=F32)
        return m, l, acc

    def att(h, e, filler):
        flat = []
        for i in range(S // BQ):
            kend = (i + 1) * BQ
            flat += [(i, k0, min(BK, kend - k0), k0 + BK >= kend) for k0 in range(0, kend, BK)]
        st = None
        pend = []

        def retire(st):
            i, k0, w, last, s = pend.pop(0)
            st = upd(e, st, k0, w, s)
            if last:
                _, l, acc = st
                ctx = (acc / l).astype(BF16)
                acc_s[pl.ds(i * BQ, BQ), :] += lax.dot_general(ctx, woT_s[h], NT, preferred_element_type=F32)
                filler(i)
                st = None
            return st

        for (i, k0, w, last) in flat:
            pend.append((i, k0, w, last, qk(e, i, k0, w)))
            if len(pend) > 1:
                st = retire(st)
        while pend:
            st = retire(st)

    NB = S // BQ
    prep_a(0, 0, 0)
    for r in range(NB):
        proj(0, r, BQ)

    def pair(p, carry):
        pair_wait(p, b_dst, bwoT_s, sem_b)

        @pl.when(p < NP - 2)
        def _():
            for cp in pair_copies(p + 2, b_src, b_dst, bwoT_h, bwoT_s, sem_b):
                cp.start()

        @pl.when(p < NP - 3)
        def _():
            for cp in pair_copies(p + 3, a_src, a_dst, woT_h, woT_s, sem_a):
                cp.start()

        @pl.when(p == NP - 2)
        def _():
            for cp in misc[2:]:
                cp.start()

        h = 2 * p
        prep_a(h + 1, p, 1)
        prep_b(h, p, 0)
        att(h, 0, lambda i: proj(1, i, BQ))

        @pl.when(p < NP - 1)
        def _():
            pair_wait(p + 1, a_dst, woT_s, sem_a)

        prep_a(h + 2, jnp.minimum(p + 1, NP - 1), 0)
        prep_b(h + 1, p, 1)
        att(h + 1, 1, lambda i: proj(0, i, BQ))
        return carry

    with jax.named_scope('Aloop'):
        lax.fori_loop(0, NP, pair, 0)
    misc[2].wait()
    misc[3].wait()
    for i in range(NB):
        rows = pl.ds(i * BQ, BQ)
        xb_s[rows, :] = xT_s[1, :, rows].T
        out_s[rows, 0:DM] = acc_s[rows, :].astype(BF16)

    L = NMEM + seg
    ri = lax.broadcasted_iota(jnp.int32, (L, L), 0)
    ci = lax.broadcasted_iota(jnp.int32, (L, L), 1)
    mask = (ri < NMEM) | (ri >= ci)

    def step(t, mem):
        rows = pl.ds(pl.multiple_of(t * seg, seg), seg)
        hcat = jnp.concatenate([mem, xb_s[rows, :].astype(F32)], axis=0)

        def pj(g):
            cols = pl.ds(g * GW, GW)
            qkv_s[:, cols] = lax.dot_general(hcat, bw_s[:, cols], NN, preferred_element_type=F32)

        def at(g):
            for j in range(HG):
                q = _r16(qkv_s[:, pl.ds(g * GW + j * DH, DH)] * QSCALE)
                k = _r16(qkv_s[:, pl.ds(g * GW + (HG + j) * DH, DH)])
                v = _r16(qkv_s[:, pl.ds(g * GW + (2 * HG + j) * DH, DH)])
                s = lax.dot_general(q, k, NT, preferred_element_type=F32)
                s = jnp.where(mask, s, NEG)
                m = jnp.max(s, axis=1, keepdims=True)
                p = jnp.exp2(s - m)
                l = jnp.sum(p, axis=1, keepdims=True)
                o = jnp.dot(_r16(p), v, preferred_element_type=F32) / l
                ob_s[:, pl.ds((g * HG + j) * DH, DH)] = _r16(o)

        def op(g):
            sl = pl.ds(g * HG * DH, HG * DH)
            return lax.dot_general(ob_s[:, sl], bwo_s[sl, :], NN, preferred_element_type=F32)

        out = None
        for g in range(G + 2):
            if g < G:
                pj(g)
            if 0 <= g - 1 < G:
                at(g - 1)
            if 0 <= g - 2 < G:
                r = op(g - 2)
                out = r if out is None else out + r
        out = out.astype(BF16)
        out_s[rows, DM:2 * DM] = out[NMEM:, :]

        @pl.when(t % OC == OC - 1)
        def _():
            out_copy(t // OC).start()
        return out[:NMEM, :].astype(F32)

    OC = 4

    def out_copy(c):
        rows = pl.ds(pl.multiple_of(c * (OC * seg), OC * seg), OC * seg)
        return pltpu.make_async_copy(out_s.at[rows, :], o_h.at[rows, :], sem_o.at[c])

    with jax.named_scope('Bloop'):
        lax.fori_loop(0, S // seg, step, mem0_s[...].astype(F32), unroll=2)
    for c in range(S // seg // OC):
        out_copy(c).wait()


@functools.partial(jax.jit, static_argnames=("B_seg_len",))
def pallas_concat_heads__compressed_kv_cla__memory_aug_recurrent_mem_tr__prompt_kernel(
        A_x, A_c_kv, A_w_q, A_w_uk, A_w_uv, A_w_o,
        B_x, B_mem0, B_Wq, B_Wk, B_Wv, B_Wo, B_seg_len):
    seg = int(B_seg_len)
    L = NMEM + seg
    vm = pl.BlockSpec(memory_space=pltpu.VMEM)
    hbm = pl.BlockSpec(memory_space=pl.ANY)
    NP = H // 2
    out = pl.pallas_call(
        functools.partial(_kernel, seg=seg),
        out_shape=jax.ShapeDtypeStruct((S, 2 * DM), BF16),
        in_specs=[hbm] * 12,
        out_specs=hbm,
        scratch_shapes=[
            pltpu.VMEM((2, DM, S), BF16),
            pltpu.VMEM((S, DM), BF16),
            pltpu.VMEM((S, DM), BF16),
            pltpu.VMEM((S, DC), BF16),
            pltpu.VMEM((H, DM, DH), BF16),
            pltpu.VMEM((H, DM, DH), BF16),
            pltpu.VMEM((NMEM, DM), BF16),
            pltpu.VMEM((NP, DM, DH), U32),
            pltpu.VMEM((NP, DC, DH), U32),
            pltpu.VMEM((NP, DC, DH), U32),
            pltpu.VMEM((NP, DM, DH), U32),
            pltpu.VMEM((NP, DM, DH), U32),
            pltpu.VMEM((NP, DM, DH), U32),
            pltpu.VMEM((2, DM, DH), BF16),
            pltpu.VMEM((2, DC, 2 * DH), BF16),
            pltpu.VMEM((2, S, DH), BF16),
            pltpu.VMEM((2, S, DH), BF16),
            pltpu.VMEM((2, S, DH), BF16),
            pltpu.VMEM((S, DM), F32),
            pltpu.VMEM((DM, 3 * H * DH), BF16),
            pltpu.VMEM((H * DH, DM), BF16),
            pltpu.VMEM((L, 3 * H * DH), F32),
            pltpu.VMEM((L, H * DH), F32),
            pltpu.VMEM((S, 2 * DM), BF16),
            pltpu.SemaphoreType.DMA((NP,)),
            pltpu.SemaphoreType.DMA((NP,)),
            pltpu.SemaphoreType.DMA((4,)),
            pltpu.SemaphoreType.DMA((S // seg // 4,)),
        ],
        compiler_params=pltpu.CompilerParams(vmem_limit_bytes=124 * 2 ** 20),
    )(jnp.swapaxes(A_x, 1, 2).reshape(DM, S), A_c_kv.reshape(S, DC),
      A_w_q, A_w_uk, A_w_uv, jnp.swapaxes(A_w_o, 1, 2),
      jnp.swapaxes(B_x, 1, 2).reshape(DM, S), B_mem0.reshape(NMEM, DM),
      B_Wq, B_Wk, B_Wv, jnp.swapaxes(B_Wo, 1, 2))
    return out.reshape(1, S, 2 * DM)
```
